```python
import jax
import jax.numpy as jnp

def _softmax(x, axis=-1):
    return jax.nn.softmax(x, axis=axis)
def _gelu(x):
    return jax.nn.gelu(x, approximate=True)
def _silu(x):
    return jax.nn.silu(x)
def _sigmoid(x):
    return jax.nn.sigmoid(x)
def _layernorm(x, axis=-1, eps=1e-5):
    m = jnp.mean(x, axis=axis, keepdims=True)
    v = jnp.var(x, axis=axis, keepdims=True)
    return (x - m) / jnp.sqrt(v + eps)
def _scatter_add(tgt, idx, src, axis=0):
    return tgt.at[idx].add(src)
def _segment_sum(src, seg, n):
    return jax.ops.segment_sum(src, seg, n)
class _Rng:
    def __init__(self, key):
        self._k = key
    def _next(self):
        self._k, sub = jax.random.split(self._k)
        return sub
    def normal(self, shape):
        return jax.random.normal(self._next(), shape, dtype=jnp.bfloat16)
    def randint(self, lo, hi, shape):
        return jax.random.randint(self._next(), shape, lo, hi, dtype=jnp.int32)
    def uniform(self, shape, lo=0.0, hi=1.0):
        return jax.random.uniform(self._next(), shape, jnp.bfloat16, lo, hi)
    def permutation(self, n):
        return jax.random.permutation(self._next(), n)


kernel_name = 'recurrent_scan__sliding_block_cached__moe_arch_mod__prompt'

def setup_inputs():
    _rng = _Rng(jax.random.key(int.from_bytes(__import__("os").urandom(4), "little")))
    _w = (lambda a: (lambda t: t.astype(jnp.bfloat16) if jnp.issubdtype(t.dtype, jnp.floating) else t)(jnp.asarray(a)))
    def _A_setup():
        B, Sq, D = 1, 2048, 640
        Hq, Hkv, Sk, Dh = 32, 32, 2048, 192
        assert Hq % Hkv == 0, (Hq, Hkv)
        return {
            "x": _w((lambda *s: _rng.normal(s) * 0.05)(B, Sq, D)),
            "k_cache": _w((lambda *s: _rng.normal(s) * 0.05)(B, Hkv, Sk, Dh)),
            "v_cache": _w((lambda *s: _rng.normal(s) * 0.05)(B, Hkv, Sk, Dh)),
            "wq": _w((lambda *s: _rng.normal(s) * 0.05)(D, Hq * Dh) * (D ** -0.5)),
            "wo": _w((lambda *s: _rng.normal(s) * 0.05)(Hq * Dh, D) * ((Hq * Dh) ** -0.5)),
        }
    _A_in = _A_setup()

    def _B_setup():
        B, S, D, F, C = 1, 2048, 640, 1536, 2
        return {
            "x": _w((lambda *s: _rng.normal(s) * 0.05)(B, S, D)),
            "w_r": _w((lambda *s: _rng.normal(s) * 0.05)(D)),
            "w_gate": _w((lambda *s: _rng.normal(s) * 0.05)(D, F)),
            "w_up": _w((lambda *s: _rng.normal(s) * 0.05)(D, F)),
            "w_down": _w((lambda *s: _rng.normal(s) * 0.05)(F, D)),
        }
    _B_in = _B_setup()

    return {
        "A_x": _A_in["x"],
        "A_k_cache": _A_in["k_cache"],
        "A_v_cache": _A_in["v_cache"],
        "A_wq": _A_in["wq"],
        "A_wo": _A_in["wo"],
        "B_x": _B_in["x"],
        "B_w_r": _B_in["w_r"],
        "B_w_gate": _B_in["w_gate"],
        "B_w_up": _B_in["w_up"],
        "B_w_down": _B_in["w_down"],
    }

def reference(A_x, A_k_cache, A_v_cache, A_wq, A_wo, B_x, B_w_r, B_w_gate, B_w_up, B_w_down):
    def _A_ref(x, k_cache, v_cache, wq, wo):
        B, Sq, D = x.shape
        Hq, Dh = 32, 192
        Hkv, Sk = k_cache.shape[1], k_cache.shape[2]
        W = min(4096, max(256, Sk // 4))
        rep = Hq // Hkv
        q = (lambda x, *d: x.transpose(*d))((x @ wq).reshape(B, Sq, Hq, Dh), 0, 2, 1, 3)
        k = jnp.repeat(k_cache[:, :, Sk - W:, :], rep, axis=1)
        v = jnp.repeat(v_cache[:, :, Sk - W:, :], rep, axis=1)
        scores = jnp.einsum("bhqd,bhkd->bhqk", q, k) * (Dh ** -0.5)
        p = _softmax(scores, axis=-1)
        o = jnp.einsum("bhqk,bhkd->bhqd", p, v)
        return (lambda x, *d: x.transpose(*d))(o, 0, 2, 1, 3).reshape(B, Sq, Hq * Dh) @ wo

    def _B_ref(x, w_r, w_gate, w_up, w_down):
        B, S, D = x.shape
        C = 2
        r = x @ w_r
        idx = jnp.argsort(-r, axis=-1)[:, :C]
        idx_e = jnp.repeat(idx.reshape(B, C, 1), D, axis=2)
        x_sel = jnp.take_along_axis(x, idx_e, axis=1)
        g = _silu(x_sel @ w_gate)
        u = x_sel @ w_up
        y = (g * u) @ w_down
        r_sel = _sigmoid(jnp.take_along_axis(r, idx, axis=1))
        y = y * r_sel.reshape(B, C, 1)
        b_off = (jnp.arange(B) * S).reshape(B, 1)
        flat_idx = (idx + b_off).reshape(B * C)
        zero = (x * 0.0).reshape(B * S, D)
        upd = _scatter_add(zero, flat_idx, y.reshape(B * C, D), axis=0)
        return x + upd.reshape(B, S, D)

    x = A_x
    xn = _layernorm(x, axis=-1)
    s = _A_ref(xn, A_k_cache, A_v_cache, A_wq, A_wo)
    g = _silu(_B_ref(xn, B_w_r, B_w_gate, B_w_up, B_w_down))
    return x + s * g
```

```python
import functools
import math

import jax
import jax.numpy as jnp
from jax import lax
import jax.experimental.pallas as pl
import jax.experimental.pallas.tpu as pltpu

S = 2048
D = 640
H = 32
DH = 192
W = 512
F = 1536
G = 2
NP = H // G
LOG2E = 1.4426950408889634

bf16 = jnp.bfloat16
f32 = jnp.float32

NT = (((1,), (1,)), ((), ()))
TN = (((0,), (0,)), ((), ()))


def _rb(x):
    return x.astype(bf16).astype(f32)


def _silu(x):
    return x / (1.0 + jnp.exp(-x))


def make_kernel(TQ=512, vmem_mb=100, unroll=True):
    NQ = S // TQ

    def kernel(x_ref, kt_ref, vt_ref, wq_ref, wo_ref, wr_ref, wg_ref, wu_ref, wd_ref,
               o_ref, xn_ref, acc_ref, k_scr, wot_scr, y_scr, idx_scr):
        p = pl.program_id(0)

        @pl.when(p == 0)
        def _prologue():
            RB = 256
            wr = wr_ref[...].astype(f32)
            best1 = best2 = None
            rs = []
            for i in range(S // RB):
                x = x_ref[i * RB:(i + 1) * RB, :].astype(f32)
                m = jnp.mean(x, axis=-1, keepdims=True)
                xc = x - m
                v = jnp.mean(xc * xc, axis=-1, keepdims=True)
                mb = _rb(m)
                vb = _rb(v)
                den = _rb(jnp.sqrt(_rb(vb + EPS_B)))
                xn = _rb(_rb(x - mb) / den)
                xn_ref[i * RB:(i + 1) * RB, :] = xn.astype(bf16)
                rs.append(_rb(jnp.sum(xn * wr, axis=-1, keepdims=True)))
            r = jnp.concatenate(rs, axis=0)
            row = lax.broadcasted_iota(jnp.int32, (S, 1), 0)
            m1 = jnp.max(r)
            i1 = jnp.min(jnp.where(r == m1, row, S))
            r2 = jnp.where(row == i1, -jnp.inf, r)
            m2 = jnp.max(r2)
            i2 = jnp.min(jnp.where(r2 == m2, row, S))
            idx_scr[0] = i1
            idx_scr[1] = i2
            sub = lax.broadcasted_iota(jnp.int32, (16, 1), 0)
            a1 = pl.multiple_of((i1 // 16) * 16, 16)
            a2 = pl.multiple_of((i2 // 16) * 16, 16)
            c1 = xn_ref[pl.ds(a1, 16), :].astype(f32)
            c2 = xn_ref[pl.ds(a2, 16), :].astype(f32)
            x1 = jnp.sum(jnp.where(sub == i1 - a1, c1, 0.0), axis=0, keepdims=True)
            x2 = jnp.sum(jnp.where(sub == i2 - a2, c2, 0.0), axis=0, keepdims=True)
            xs = jnp.where(sub == 0, x1, jnp.where(sub == 1, x2, 0.0)).astype(bf16)
            gt = _rb(jnp.dot(xs, wg_ref[...], preferred_element_type=f32))
            up = _rb(jnp.dot(xs, wu_ref[...], preferred_element_type=f32))
            hmid = _rb(_rb(_silu(gt)) * up).astype(bf16)
            y = _rb(jnp.dot(hmid, wd_ref[...], preferred_element_type=f32))
            rsel = jnp.where(sub == 0, m1, m2)
            sig = _rb(1.0 / (1.0 + jnp.exp(-rsel)))
            y_scr[...] = _rb(y * sig)
            acc_ref[...] = jnp.zeros_like(acc_ref)

        z = jnp.zeros((64, W), bf16)
        k_scr[0] = jnp.concatenate([kt_ref[0], z], axis=0).T
        k_scr[1] = jnp.concatenate([z, kt_ref[1]], axis=0).T
        wot_scr[...] = wo_ref[...].T

        qscale = (DH ** -0.5) * LOG2E

        def tile(t):
            off = t * TQ if isinstance(t, int) else pl.multiple_of(t * TQ, TQ)
            xn = xn_ref[pl.ds(off, TQ), :]
            q = (jnp.dot(xn, wq_ref[...], preferred_element_type=f32) * qscale).astype(bf16)
            os_ = []
            for h in range(G):
                qh = q[:, 128 * h:128 * h + 256]
                st = lax.dot_general(k_scr[h], qh, NT, preferred_element_type=f32)
                mx = jnp.max(st, axis=0, keepdims=True)
                pt = jnp.exp2(st - mx)
                l = jnp.sum(pt, axis=0, keepdims=True)
                ot = jnp.dot(vt_ref[h], pt.astype(bf16), preferred_element_type=f32)
                os_.append((ot * (1.0 / l)).astype(bf16))
            ot2 = jnp.concatenate(os_, axis=0)
            acc_ref[:, pl.ds(off, TQ)] += jnp.dot(wot_scr[...], ot2, preferred_element_type=f32)

        if unroll:
            for t in range(NQ):
                tile(t)
        else:
            lax.fori_loop(0, NQ, lambda t, c: (tile(t), c)[1], 0)

        @pl.when(p == NP - 1)
        def _epilogue():
            RB = 256
            i1 = idx_scr[0]
            i2 = idx_scr[1]
            y1 = y_scr[0:1, :]
            y2 = y_scr[1:2, :]
            for i in range(S // RB):
                s = _rb(acc_ref[:, i * RB:(i + 1) * RB].T)
                xn = xn_ref[i * RB:(i + 1) * RB, :].astype(f32)
                row = lax.broadcasted_iota(jnp.int32, (RB, 1), 0) + i * RB
                u = jnp.where(row == i1, y1, jnp.where(row == i2, y2, 0.0))
                g = _rb(_silu(_rb(xn + u)))
                x = x_ref[i * RB:(i + 1) * RB, :].astype(f32)
                o_ref[i * RB:(i + 1) * RB, :] = (x + _rb(s * g)).astype(o_ref.dtype)

    @jax.jit
    def run(A_x, A_k_cache, A_v_cache, A_wq, A_wo, B_x, B_w_r, B_w_gate, B_w_up, B_w_down):
        x = A_x.reshape(S, D)
        kt = jnp.swapaxes(A_k_cache, 2, 3).reshape(H, DH, S)
        vt = jnp.swapaxes(A_v_cache, 2, 3).reshape(H, DH, S)
        wr = B_w_r.reshape(1, D)
        const = lambda p: (0, 0)
        out = pl.pallas_call(
            kernel,
            grid=(NP,),
            in_specs=[
                pl.BlockSpec((S, D), const),
                pl.BlockSpec((G, DH, W), lambda p: (p, 0, S // W - 1)),
                pl.BlockSpec((G, DH, W), lambda p: (p, 0, S // W - 1)),
                pl.BlockSpec((D, G * DH), lambda p: (0, p)),
                pl.BlockSpec((G * DH, D), lambda p: (p, 0)),
                pl.BlockSpec((1, D), const),
                pl.BlockSpec((D, F), const),
                pl.BlockSpec((D, F), const),
                pl.BlockSpec((F, D), const),
            ],
            out_specs=pl.BlockSpec((S, D), const),
            out_shape=jax.ShapeDtypeStruct((S, D), bf16),
            scratch_shapes=[
                pltpu.VMEM((S, D), bf16),
                pltpu.VMEM((D, S), f32),
                pltpu.VMEM((G, W, 256), bf16),
                pltpu.VMEM((D, G * DH), bf16),
                pltpu.VMEM((16, D), f32),
                pltpu.SMEM((2,), jnp.int32),
            ],
            compiler_params=pltpu.CompilerParams(
                dimension_semantics=("arbitrary",),
                vmem_limit_bytes=vmem_mb * 1024 * 1024),
        )(x, kt, vt, A_wq, A_wo, wr, B_w_gate, B_w_up, B_w_down)
        return out.reshape(1, S, D)

    return run


import numpy as np
import ml_dtypes
EPS_B = float(np.float32(np.asarray(1e-5, dtype=ml_dtypes.bfloat16)))

pallas_recurrent_scan__sliding_block_cached__moe_arch_mod__prompt_kernel = make_kernel()
```

```python
import jax
import jax.numpy as jnp
from jax import lax
import jax.experimental.pallas as pl
import jax.experimental.pallas.tpu as pltpu
import ml_dtypes
import numpy as np

S = 2048
D = 640
H = 32
DH = 192
W = 512
F = 1536
G = 2
NP = H // G
LOG2E = 1.4426950408889634
EPS_B = float(np.float32(np.asarray(1e-5, dtype=ml_dtypes.bfloat16)))

bf16 = jnp.bfloat16
f32 = jnp.float32

NT = (((1,), (1,)), ((), ()))


def _rb(x):
    return x.astype(bf16).astype(f32)


def _sigmoid(x):
    e = jnp.exp(jnp.minimum(-x, 80.0))
    d = 1.0 + e
    r = pl.reciprocal(d, approx=True)
    return r * (2.0 - d * r)


def make_kernel(TQ=1024, vmem_mb=100, order=1, gpos=0, TX=512, TO=256, ffn_step=2):
    NQ = S // TQ
    NX = S // TX
    NO = S // TO

    def kernel(x_hbm, kt_ref, vt_ref, wq_ref, wo_ref, wr_ref, wg_hbm, wu_hbm, wd_hbm,
               o_hbm, x_scr, xn_ref, acc_ref, k_scr, wot_scr, r_scr, y_scr, wg_scr, wu_scr, wd_scr,
               o_scr, g_scr, idx_scr, xsem, wsem, osem):
        p = pl.program_id(0)

        def x_copy(t):
            return pltpu.make_async_copy(x_hbm.at[pl.ds(t * TX, TX)], x_scr.at[pl.ds(t * TX, TX)], xsem.at[t])

        def o_copy(t):
            return pltpu.make_async_copy(o_scr.at[pl.ds(t * TO, TO)], o_hbm.at[pl.ds(t * TO, TO)], osem.at[t])

        def w_copies():
            return [pltpu.make_async_copy(a, b, wsem.at[i])
                    for i, (a, b) in enumerate(((wg_hbm, wg_scr), (wu_hbm, wu_scr), (wd_hbm, wd_scr)))]

        @pl.when(p == 0)
        def _():
            for t in range(NX):
                x_copy(t).start()

        qscale = (DH ** -0.5) * LOG2E

        def sl(t):
            return pl.ds(t * TQ, TQ)

        def layernorm(t):
            x_copy(t).wait()
            x = x_scr[pl.ds(t * TX, TX), :].astype(f32)
            m = jnp.mean(x, axis=-1, keepdims=True)
            xc = x - m
            v = jnp.mean(xc * xc, axis=-1, keepdims=True)
            xn = xc * lax.rsqrt(v + 1e-5)
            xn_ref[pl.ds(t * TX, TX), :] = xn.astype(bf16)
            r = jnp.sum(xn * wr_ref[...].astype(f32), axis=-1, keepdims=True)
            lane = lax.broadcasted_iota(jnp.int32, (8, 128), 1)
            rm = jnp.full((8, 128), -jnp.inf, f32)
            for j in range(TX // 8):
                rm = jnp.where(lane == j, r[8 * j:8 * j + 8, :], rm)
            r_scr[t] = rm

        def route_and_ffn():
            for c in w_copies():
                c.wait()
            r = r_scr[...]
            shp = (NX, 8, 128)
            row = (lax.broadcasted_iota(jnp.int32, shp, 0) * TX
                   + lax.broadcasted_iota(jnp.int32, shp, 2) * 8
                   + lax.broadcasted_iota(jnp.int32, shp, 1))
            m1 = jnp.max(r)
            i1 = jnp.min(jnp.where(r == m1, row, S - 1))
            r2 = jnp.where(row == i1, -jnp.inf, r)
            m2 = jnp.max(r2)
            i2 = jnp.min(jnp.where(r2 == m2, row, S - 1))
            idx_scr[0] = i1
            idx_scr[1] = i2
            sub = lax.broadcasted_iota(jnp.int32, (16, 1), 0)
            a1 = pl.multiple_of((i1 // 16) * 16, 16)
            a2 = pl.multiple_of((i2 // 16) * 16, 16)
            c1 = xn_ref[pl.ds(a1, 16), :].astype(f32)
            c2 = xn_ref[pl.ds(a2, 16), :].astype(f32)
            x1 = jnp.sum(jnp.where(sub == i1 - a1, c1, 0.0), axis=0, keepdims=True)
            x2 = jnp.sum(jnp.where(sub == i2 - a2, c2, 0.0), axis=0, keepdims=True)
            xs = jnp.where(sub == 0, x1, jnp.where(sub == 1, x2, 0.0)).astype(bf16)
            gt = _rb(jnp.dot(xs, wg_scr[...], preferred_element_type=f32))
            up = _rb(jnp.dot(xs, wu_scr[...], preferred_element_type=f32))
            hmid = _rb(_rb(gt * _sigmoid(gt)) * up).astype(bf16)
            y = _rb(jnp.dot(hmid, wd_scr[...], preferred_element_type=f32))
            sig = _rb(_sigmoid(jnp.where(sub == 0, m1, m2)))
            y_scr[...] = _rb(y * sig)

        GR = S // NP

        def gate_chunk(off):
            xn = xn_ref[pl.ds(off, GR), :].astype(f32)
            row = lax.broadcasted_iota(jnp.int32, (GR, 1), 0) + off
            u = jnp.where(row == idx_scr[0], y_scr[0:1, :], jnp.where(row == idx_scr[1], y_scr[1:2, :], 0.0))
            z = xn + u
            g_scr[pl.ds(off, GR), :] = (z * _sigmoid(z)).astype(bf16)

        def epilogue(t):
            s = acc_ref[:, pl.ds(t * TO, TO)].T
            x = x_scr[pl.ds(t * TO, TO), :].astype(f32)
            o_scr[pl.ds(t * TO, TO), :] = (x + s * g_scr[pl.ds(t * TO, TO), :].astype(f32)).astype(bf16)
            o_copy(t).start()

        def step(first, last):
            z = jnp.zeros((64, W), bf16)
            k_scr[0] = jnp.concatenate([kt_ref[0], z], axis=0).T
            k_scr[1] = jnp.concatenate([z, kt_ref[1]], axis=0).T
            wot_scr[...] = wo_ref[...].T

            def qproj(t):
                xn = xn_ref[sl(t), :]
                return (jnp.dot(xn, wq_ref[...], preferred_element_type=f32) * qscale).astype(bf16)

            def qk(q, h):
                return lax.dot_general(k_scr[h], q[:, 128 * h:128 * h + 256], NT, preferred_element_type=f32)

            def sm(st):
                mx = jnp.max(st, axis=0, keepdims=True)
                pt = jnp.exp2(st - mx)
                l = jnp.sum(pt, axis=0, keepdims=True)
                return pt.astype(bf16), 1.0 / l

            def pv(pl_, h):
                pt, rl = pl_
                return (jnp.dot(vt_ref[h], pt, preferred_element_type=f32) * rl).astype(bf16)

            def oproj(t, o0, o1):
                ot2 = jnp.concatenate([o0, o1], axis=0)
                a = jnp.dot(wot_scr[...], ot2, preferred_element_type=f32)
                acc_ref[:, sl(t)] += a

            if order == 1:
                for t in range(NQ):
                    q = qproj(t)
                    s0 = qk(q, 0); s1 = qk(q, 1)
                    if t == gpos:
                        gate_chunk(pl.multiple_of(p * GR, GR))
                    o0 = pv(sm(s0), 0)
                    o1 = pv(sm(s1), 1)
                    oproj(t, o0, o1)
            elif order == 0:
                for t in range(NQ):
                    q = qproj(t)
                    if t == gpos:
                        gate_chunk(pl.multiple_of(p * GR, GR))
                    o = [pv(sm(qk(q, h)), h) for h in range(2)]
                    oproj(t, *o)
            elif order == 3:
                qs = [qproj(t) for t in range(NQ)]
                gate_chunk(pl.multiple_of(p * GR, GR))
                for t in range(NQ):
                    s0 = qk(qs[t], 0); s1 = qk(qs[t], 1)
                    o0 = pv(sm(s0), 0)
                    o1 = pv(sm(s1), 1)
                    oproj(t, o0, o1)
            elif order == 4:
                qs = [qproj(t) for t in range(NQ)]
                gate_chunk(pl.multiple_of(p * GR, GR))
                os_ = []
                for t in range(NQ):
                    s0 = qk(qs[t], 0); s1 = qk(qs[t], 1)
                    o0 = pv(sm(s0), 0)
                    o1 = pv(sm(s1), 1)
                    os_.append((o0, o1))
                for t in range(NQ):
                    oproj(t, *os_[t])
            elif order == 2:
                q = qproj(0)
                prev = None
                for t in range(NQ):
                    s0 = qk(q, 0); s1 = qk(q, 1)
                    if t == gpos:
                        gate_chunk(pl.multiple_of(p * GR, GR))
                    p0 = sm(s0)
                    if prev is not None:
                        oproj(t - 1, *prev)
                    o0 = pv(p0, 0)
                    p1 = sm(s1)
                    if t + 1 < NQ:
                        q = qproj(t + 1)
                    o1 = pv(p1, 1)
                    prev = (o0, o1)
                oproj(NQ - 1, *prev)

        @pl.when(p == 0)
        def _():
            for t in range(NX):
                layernorm(t)
            for c in w_copies():
                c.start()
            acc_ref[...] = jnp.zeros_like(acc_ref)
            idx_scr[0] = -1
            idx_scr[1] = -1
            y_scr[...] = jnp.zeros_like(y_scr)

        @pl.when(p == ffn_step)
        def _():
            route_and_ffn()
            for i in range(ffn_step):
                gate_chunk(i * GR)

        step(False, False)

        @pl.when(p == NP - 1)
        def _():
            for t in range(NO):
                epilogue(t)
            for t in range(NO):
                o_copy(t).wait()

    @jax.jit
    def run(A_x, A_k_cache, A_v_cache, A_wq, A_wo, B_x, B_w_r, B_w_gate, B_w_up, B_w_down):
        x = A_x.reshape(S, D)
        kt = jnp.swapaxes(A_k_cache, 2, 3).reshape(H, DH, S)
        vt = jnp.swapaxes(A_v_cache, 2, 3).reshape(H, DH, S)
        wr = B_w_r.reshape(1, D)
        const = lambda p: (0, 0)
        anyspec = pl.BlockSpec(memory_space=pl.ANY)
        out = pl.pallas_call(
            kernel,
            grid=(NP,),
            in_specs=[
                anyspec,
                pl.BlockSpec((G, DH, W), lambda p: (p, 0, S // W - 1)),
                pl.BlockSpec((G, DH, W), lambda p: (p, 0, S // W - 1)),
                pl.BlockSpec((D, G * DH), lambda p: (0, p)),
                pl.BlockSpec((G * DH, D), lambda p: (p, 0)),
                pl.BlockSpec((1, D), const),
                anyspec, anyspec, anyspec,
            ],
            out_specs=anyspec,
            out_shape=jax.ShapeDtypeStruct((S, D), bf16),
            scratch_shapes=[
                pltpu.VMEM((S, D), bf16),
                pltpu.VMEM((S, D), bf16),
                pltpu.VMEM((D, S), f32),
                pltpu.VMEM((G, W, 256), bf16),
                pltpu.VMEM((D, G * DH), bf16),
                pltpu.VMEM((NX, 8, 128), f32),
                pltpu.VMEM((16, D), f32),
                pltpu.VMEM((D, F), bf16),
                pltpu.VMEM((D, F), bf16),
                pltpu.VMEM((F, D), bf16),
                pltpu.VMEM((S, D), bf16),
                pltpu.VMEM((S, D), bf16),
                pltpu.SMEM((2,), jnp.int32),
                pltpu.SemaphoreType.DMA((NX,)),
                pltpu.SemaphoreType.DMA((3,)),
                pltpu.SemaphoreType.DMA((NO,)),
            ],
            compiler_params=pltpu.CompilerParams(
                dimension_semantics=("arbitrary",),
                vmem_limit_bytes=vmem_mb * 1024 * 1024),
        )(x, kt, vt, A_wq, A_wo, wr, B_w_gate, B_w_up, B_w_down)
        return out.reshape(1, S, D)

    return run


pallas_recurrent_scan__sliding_block_cached__moe_arch_mod__prompt_kernel = make_kernel(TX=256, TO=128, ffn_step=1)
```

```python
import jax
import jax.numpy as jnp
from jax import lax
import jax.experimental.pallas as pl
import jax.experimental.pallas.tpu as pltpu

S = 2048
D = 640
H = 32
DH = 192
W = 512
F = 1536
G = 2
NP = H // G
LOG2E = 1.4426950408889634

bf16 = jnp.bfloat16
f32 = jnp.float32

NT = (((1,), (1,)), ((), ()))


def _sigmoid(x):
    e = jnp.exp(jnp.minimum(-x, 80.0))
    d = 1.0 + e
    r = pl.reciprocal(d, approx=True)
    return r * (2.0 - d * r)


def make_kernel(TQ=1024, vmem_mb=100, sched=None, TX=256, RC=32, TO=128, ffn_step=1, flags=None):
    NQ = S // TQ
    NX = S // TX
    NO = S // TO

    def kernel(x_hbm, kt_hbm, vt_hbm, wq_hbm, wo_hbm, wr_ref, wg_hbm, wu_hbm, wd_hbm,
               o_hbm, x_scr, xn_ref, g_scr, acc_ref, kt_buf, vt_buf, wq_buf, wo_buf, k_scr, wot_scr,
               r_scr, wg_scr, wu_scr, wd_scr, o_scr, xsem, bsem, wsem, osem):
        p = pl.program_id(0)
        slot = p % 2

        def x_copy(t):
            return pltpu.make_async_copy(x_hbm.at[pl.ds(t * TX, TX)], x_scr.at[pl.ds(t * TX, TX)], xsem.at[t])

        def o_copy(t):
            return pltpu.make_async_copy(o_scr.at[pl.ds(t * TO, TO)], o_hbm.at[pl.ds(t * TO, TO)], osem.at[t])

        def w_copies():
            return [pltpu.make_async_copy(a, b, wsem.at[i])
                    for i, (a, b) in enumerate(((wg_hbm, wg_scr), (wu_hbm, wu_scr), (wd_hbm, wd_scr)))]

        def b_copies(q, s):
            hs = pl.ds(q * G, G)
            cs = pl.ds(pl.multiple_of(q * (G * DH), G * DH), G * DH)
            ws = pl.ds(S - W, W)
            return [
                pltpu.make_async_copy(wq_hbm.at[:, cs], wq_buf.at[s], bsem.at[s, 0]),
                pltpu.make_async_copy(kt_hbm.at[hs, :, ws], kt_buf.at[s], bsem.at[s, 1]),
                pltpu.make_async_copy(vt_hbm.at[hs, :, ws], vt_buf.at[s], bsem.at[s, 2]),
                pltpu.make_async_copy(wo_hbm.at[cs, :], wo_buf.at[s], bsem.at[s, 3]),
            ]

        def layernorm(t):
            x_copy(t).wait()
            wr = wr_ref[...].astype(f32)
            lane = lax.broadcasted_iota(jnp.int32, (8, 128), 1)
            rm = jnp.full((8, 128), -jnp.inf, f32)
            for c in range(TX // RC):
                rows = pl.ds(t * TX + c * RC, RC)
                x = x_scr[rows, :].astype(f32)
                m = jnp.mean(x, axis=-1, keepdims=True)
                xc = x - m
                v = jnp.mean(xc * xc, axis=-1, keepdims=True)
                xn = xc * lax.rsqrt(v + 1e-5)
                xn_ref[rows, :] = xn.astype(bf16)
                g_scr[rows, :] = (xn * _sigmoid(xn)).astype(bf16)
                r = jnp.sum(xn * wr, axis=-1, keepdims=True)
                for j in range(RC // 8):
                    rm = jnp.where(lane == c * (RC // 8) + j, r[8 * j:8 * j + 8, :], rm)
            r_scr[t] = rm

        def route_and_ffn():
            for c in w_copies():
                c.wait()
            r = r_scr[...]
            shp = (NX, 8, 128)
            row = (lax.broadcasted_iota(jnp.int32, shp, 0) * TX
                   + lax.broadcasted_iota(jnp.int32, shp, 2) * 8
                   + lax.broadcasted_iota(jnp.int32, shp, 1))
            m1 = jnp.max(r)
            i1 = jnp.min(jnp.where(r == m1, row, S - 1))
            r2 = jnp.where(row == i1, -jnp.inf, r)
            m2 = jnp.max(r2)
            i2 = jnp.min(jnp.where(r2 == m2, row, S - 1))
            sub = lax.broadcasted_iota(jnp.int32, (16, 1), 0)
            a1 = pl.multiple_of((i1 // 16) * 16, 16)
            a2 = pl.multiple_of((i2 // 16) * 16, 16)
            c1 = xn_ref[pl.ds(a1, 16), :].astype(f32)
            c2 = xn_ref[pl.ds(a2, 16), :].astype(f32)
            x1 = jnp.sum(jnp.where(sub == i1 - a1, c1, 0.0), axis=0, keepdims=True)
            x2 = jnp.sum(jnp.where(sub == i2 - a2, c2, 0.0), axis=0, keepdims=True)
            xs = jnp.where(sub == 0, x1, jnp.where(sub == 1, x2, 0.0)).astype(bf16)
            gt = jnp.dot(xs, wg_scr[...], preferred_element_type=f32)
            up = jnp.dot(xs, wu_scr[...], preferred_element_type=f32)
            hmid = (gt * _sigmoid(gt) * up).astype(bf16)
            y = jnp.dot(hmid, wd_scr[...], preferred_element_type=f32)
            y = y * _sigmoid(jnp.where(sub == 0, m1, m2))
            y1 = y[0:1, :]
            y2 = y[1:2, :]
            for a, c in ((a1, c1), (a2, c2)):
                z = c + jnp.where(sub + a == i1, y1, jnp.where(sub + a == i2, y2, 0.0))
                g_scr[pl.ds(a, 16), :] = (z * _sigmoid(z)).astype(bf16)

        def epilogue(t):
            rows = pl.ds(t * TO, TO)
            s = acc_ref[:, rows].astype(bf16).T.astype(f32)
            x = x_scr[rows, :].astype(f32)
            o_scr[rows, :] = (x + s * g_scr[rows, :].astype(f32)).astype(bf16)
            o_copy(t).start()

        qscale = (DH ** -0.5) * LOG2E

        def step():
            def sl(t):
                return pl.ds(t * TQ, TQ)

            def qproj(t):
                return (jnp.dot(xn_ref[sl(t), :], wq_buf[slot], preferred_element_type=f32) * qscale).astype(bf16)

            def qk(q, h):
                return lax.dot_general(k_scr[h], q[:, 128 * h:128 * h + 256], NT, preferred_element_type=f32)

            def sm(st):
                mx = jnp.max(st, axis=0, keepdims=True)
                pt = jnp.exp2(st - mx)
                l = jnp.sum(pt, axis=0, keepdims=True)
                return pt.astype(bf16), 1.0 / l

            def pv(pl_, h):
                pt, rl = pl_
                return (jnp.dot(vt_buf[slot, h], pt, preferred_element_type=f32) * rl).astype(bf16)

            def oproj(t, o0, o1):
                ot2 = jnp.concatenate([o0, o1], axis=0)
                acc_ref[:, sl(t)] += jnp.dot(wot_scr[...], ot2, preferred_element_type=f32)

            sc = sched
            if sc is None:
                sc = [("TK", 0), ("TK", 1), ("TW",)]
                for t in range(NQ):
                    sc += [("Q", t), ("K", t, 0), ("K", t, 1), ("S", t, 0), ("P", t, 0), ("S", t, 1), ("P", t, 1), ("O", t)]
            v = {}
            for tok in sc:
                k = tok[0]
                if k == "TK":
                    z = jnp.zeros((64, W), bf16)
                    h = tok[1]
                    k_scr[h] = (jnp.concatenate([kt_buf[slot, 0], z], axis=0) if h == 0
                                else jnp.concatenate([z, kt_buf[slot, 1]], axis=0)).T
                elif k == "TW":
                    wot_scr[...] = wo_buf[slot].T
                elif k == "Q":
                    v[tok] = qproj(tok[1])
                elif k == "K":
                    v[tok] = qk(v[("Q", tok[1])], tok[2])
                elif k == "S":
                    v[tok] = sm(v[("K",) + tok[1:]])
                elif k == "P":
                    v[tok] = pv(v[("S",) + tok[1:]], tok[2])
                elif k == "O":
                    oproj(tok[1], v[("P", tok[1], 0)], v[("P", tok[1], 1)])

        @pl.when(p == 0)
        def _():
            for t in range(NX):
                x_copy(t).start()
            for c in b_copies(0, 0):
                c.start()
            acc_ref[...] = jnp.zeros_like(acc_ref)
            for t in range(NX):
                layernorm(t)
            for c in w_copies():
                c.start()

        @pl.when(p + 1 < NP)
        def _():
            for c in b_copies(p + 1, 1 - slot):
                c.start()

        @pl.when(p == ffn_step)
        def _():
            route_and_ffn()

        for c in b_copies(p, slot):
            c.wait()

        step()

        @pl.when(p == NP - 1)
        def _():
            for t in range(NO):
                epilogue(t)
            for t in range(NO):
                o_copy(t).wait()

    @jax.jit
    def run(A_x, A_k_cache, A_v_cache, A_wq, A_wo, B_x, B_w_r, B_w_gate, B_w_up, B_w_down):
        x = A_x.reshape(S, D)
        kt = jnp.swapaxes(A_k_cache, 2, 3).reshape(H, DH, S)
        vt = jnp.swapaxes(A_v_cache, 2, 3).reshape(H, DH, S)
        wr = B_w_r.reshape(1, D)
        anyspec = pl.BlockSpec(memory_space=pl.ANY)
        out = pl.pallas_call(
            kernel,
            grid=(NP,),
            in_specs=[anyspec, anyspec, anyspec, anyspec, anyspec,
                      pl.BlockSpec((1, D), lambda p: (0, 0)),
                      anyspec, anyspec, anyspec],
            out_specs=anyspec,
            out_shape=jax.ShapeDtypeStruct((S, D), bf16),
            scratch_shapes=[
                pltpu.VMEM((S, D), bf16),
                pltpu.VMEM((S, D), bf16),
                pltpu.VMEM((S, D), bf16),
                pltpu.VMEM((D, S), f32),
                pltpu.VMEM((2, G, DH, W), bf16),
                pltpu.VMEM((2, G, DH, W), bf16),
                pltpu.VMEM((2, D, G * DH), bf16),
                pltpu.VMEM((2, G * DH, D), bf16),
                pltpu.VMEM((G, W, 256), bf16),
                pltpu.VMEM((D, G * DH), bf16),
                pltpu.VMEM((NX, 8, 128), f32),
                pltpu.VMEM((D, F), bf16),
                pltpu.VMEM((D, F), bf16),
                pltpu.VMEM((F, D), bf16),
                pltpu.VMEM((S, D), bf16),
                pltpu.SemaphoreType.DMA((NX,)),
                pltpu.SemaphoreType.DMA((2, 4)),
                pltpu.SemaphoreType.DMA((3,)),
                pltpu.SemaphoreType.DMA((NO,)),
            ],
            compiler_params=pltpu.CompilerParams(
                dimension_semantics=("arbitrary",),
                vmem_limit_bytes=vmem_mb * 1024 * 1024, flags=flags),
        )(x, kt, vt, A_wq, A_wo, wr, B_w_gate, B_w_up, B_w_down)
        return out.reshape(1, S, D)

    return run


pallas_recurrent_scan__sliding_block_cached__moe_arch_mod__prompt_kernel = make_kernel(
    flags={"XLA_TPU_FORCE_LP_LLO_SCHEDULER": True})
```

```python
import jax
import jax.numpy as jnp
from jax import lax
import jax.experimental.pallas as pl
import jax.experimental.pallas.tpu as pltpu

S = 2048
D = 640
H = 32
DH = 192
W = 512
F = 1536
G = 2
NP = H // G
LOG2E = 1.4426950408889634

bf16 = jnp.bfloat16
f32 = jnp.float32

NT = (((1,), (1,)), ((), ()))


def _sigmoid(x):
    e = jnp.exp(jnp.minimum(-x, 80.0))
    d = 1.0 + e
    r = pl.reciprocal(d, approx=True)
    return r * (2.0 - d * r)


def make_kernel(TQ=1024, vmem_mb=100, sched=None, TX=512, RC=512, TO=128, ffn_step=1, flags=None, LNU=1, WR1D=False):
    NQ = S // TQ
    NX = S // TX
    NO = S // TO

    def kernel(x_hbm, kt_hbm, vt_hbm, wq_hbm, wo_hbm, wr_ref, wg_hbm, wu_hbm, wd_hbm,
               o_hbm, x_scr, xn_ref, g_scr, acc_ref, kt_buf, vt_buf, wq_buf, wo_buf, k_scr, wot_scr,
               r_scr, wg_scr, wu_scr, wd_scr, o_scr, xsem, bsem, wsem, osem):
        p = pl.program_id(0)
        slot = p % 2

        def x_copy(t):
            return pltpu.make_async_copy(x_hbm.at[pl.ds(t * TX, TX)], x_scr.at[pl.ds(t * TX, TX)], xsem.at[t])

        def o_copy(t):
            return pltpu.make_async_copy(o_scr.at[pl.ds(t * TO, TO)], o_hbm.at[pl.ds(t * TO, TO)], osem.at[t])

        def w_copies():
            return [pltpu.make_async_copy(a, b, wsem.at[i])
                    for i, (a, b) in enumerate(((wg_hbm, wg_scr), (wu_hbm, wu_scr), (wd_hbm, wd_scr)))]

        def b_copies(q, s):
            hs = pl.ds(q * G, G)
            cs = pl.ds(pl.multiple_of(q * (G * DH), G * DH), G * DH)
            ws = pl.ds(S - W, W)
            return [
                pltpu.make_async_copy(wq_hbm.at[:, cs], wq_buf.at[s], bsem.at[s, 0]),
                pltpu.make_async_copy(kt_hbm.at[hs, :, ws], kt_buf.at[s], bsem.at[s, 1]),
                pltpu.make_async_copy(vt_hbm.at[hs, :, ws], vt_buf.at[s], bsem.at[s, 2]),
                pltpu.make_async_copy(wo_hbm.at[cs, :], wo_buf.at[s], bsem.at[s, 3]),
            ]

        def layernorm(t):
            x_copy(t).wait()
            wr = wr_ref[...].astype(f32).reshape(1, D)
            lane = lax.broadcasted_iota(jnp.int32, (8, 128), 1)

            def body(c, rm):
                rows = pl.ds(pl.multiple_of(t * TX + c * RC, RC), RC)
                x = x_scr[rows, :].astype(f32)
                m = jnp.mean(x, axis=-1, keepdims=True)
                xc = x - m
                v = jnp.mean(xc * xc, axis=-1, keepdims=True)
                xn = xc * lax.rsqrt(v + 1e-5)
                xn_ref[rows, :] = xn.astype(bf16)
                h = 0.5 * xn
                g_scr[rows, :] = (h + h * jnp.tanh(h)).astype(bf16)
                r = jnp.sum(xn * wr, axis=-1, keepdims=True)
                for j in range(RC // 8):
                    rm = jnp.where(lane == c * (RC // 8) + j, r[8 * j:8 * j + 8, :], rm)
                return rm

            r_scr[t] = lax.fori_loop(0, TX // RC, body, jnp.full((8, 128), -jnp.inf, f32), unroll=LNU)

        def route_and_ffn():
            for c in w_copies():
                c.wait()
            r = r_scr[...]
            shp = (NX, 8, 128)
            row = (lax.broadcasted_iota(jnp.int32, shp, 0) * TX
                   + lax.broadcasted_iota(jnp.int32, shp, 2) * 8
                   + lax.broadcasted_iota(jnp.int32, shp, 1))
            m1 = jnp.max(r)
            i1 = jnp.min(jnp.where(r == m1, row, S - 1))
            r2 = jnp.where(row == i1, -jnp.inf, r)
            m2 = jnp.max(r2)
            i2 = jnp.min(jnp.where(r2 == m2, row, S - 1))
            sub = lax.broadcasted_iota(jnp.int32, (16, 1), 0)
            a1 = pl.multiple_of((i1 // 16) * 16, 16)
            a2 = pl.multiple_of((i2 // 16) * 16, 16)
            c1 = xn_ref[pl.ds(a1, 16), :].astype(f32)
            c2 = xn_ref[pl.ds(a2, 16), :].astype(f32)
            x1 = jnp.sum(jnp.where(sub == i1 - a1, c1, 0.0), axis=0, keepdims=True)
            x2 = jnp.sum(jnp.where(sub == i2 - a2, c2, 0.0), axis=0, keepdims=True)
            xs = jnp.where(sub == 0, x1, jnp.where(sub == 1, x2, 0.0)).astype(bf16)
            gt = jnp.dot(xs, wg_scr[...], preferred_element_type=f32)
            up = jnp.dot(xs, wu_scr[...], preferred_element_type=f32)
            hmid = (gt * _sigmoid(gt) * up).astype(bf16)
            y = jnp.dot(hmid, wd_scr[...], preferred_element_type=f32)
            y = y * _sigmoid(jnp.where(sub == 0, m1, m2))
            y1 = y[0:1, :]
            y2 = y[1:2, :]
            for a, c in ((a1, c1), (a2, c2)):
                z = c + jnp.where(sub + a == i1, y1, jnp.where(sub + a == i2, y2, 0.0))
                g_scr[pl.ds(a, 16), :] = (z * _sigmoid(z)).astype(bf16)

        def epilogue(t):
            rows = pl.ds(t * TO, TO)
            s = acc_ref[:, rows].astype(bf16).T.astype(f32)
            x = x_scr[rows, :].astype(f32)
            o_scr[rows, :] = (x + s * g_scr[rows, :].astype(f32)).astype(bf16)
            o_copy(t).start()

        qscale = (DH ** -0.5) * LOG2E

        def step():
            def sl(t):
                return pl.ds(t * TQ, TQ)

            def qproj(t):
                return (jnp.dot(xn_ref[sl(t), :], wq_buf[slot], preferred_element_type=f32) * qscale).astype(bf16)

            def qk(q, h):
                return lax.dot_general(k_scr[h], q[:, 128 * h:128 * h + 256], NT, preferred_element_type=f32)

            def sm(st):
                mx = jnp.max(st, axis=0, keepdims=True)
                pt = jnp.exp2(st - mx)
                l = jnp.sum(pt, axis=0, keepdims=True)
                return pt.astype(bf16), 1.0 / l

            def pv(pl_, h):
                pt, rl = pl_
                return (jnp.dot(vt_buf[slot, h], pt, preferred_element_type=f32) * rl).astype(bf16)

            def oproj(t, o0, o1):
                ot2 = jnp.concatenate([o0, o1], axis=0)
                acc_ref[:, sl(t)] += jnp.dot(wot_scr[...], ot2, preferred_element_type=f32)

            sc = sched
            if sc is None:
                sc = [("TK", 0), ("TK", 1), ("TW",)]
                for t in range(NQ):
                    sc += [("Q", t), ("K", t, 0), ("K", t, 1), ("S", t, 0), ("P", t, 0), ("S", t, 1), ("P", t, 1), ("O", t)]
            v = {}
            for tok in sc:
                k = tok[0]
                if k == "TK":
                    z = jnp.zeros((64, W), bf16)
                    h = tok[1]
                    k_scr[h] = (jnp.concatenate([kt_buf[slot, 0], z], axis=0) if h == 0
                                else jnp.concatenate([z, kt_buf[slot, 1]], axis=0)).T
                elif k == "TW":
                    wot_scr[...] = wo_buf[slot].T
                elif k == "Q":
                    v[tok] = qproj(tok[1])
                elif k == "K":
                    v[tok] = qk(v[("Q", tok[1])], tok[2])
                elif k == "S":
                    v[tok] = sm(v[("K",) + tok[1:]])
                elif k == "P":
                    v[tok] = pv(v[("S",) + tok[1:]], tok[2])
                elif k == "O":
                    oproj(tok[1], v[("P", tok[1], 0)], v[("P", tok[1], 1)])

        @pl.when(p == 0)
        def _():
            for t in range(NX):
                x_copy(t).start()
            for c in b_copies(0, 0):
                c.start()
            acc_ref[...] = jnp.zeros_like(acc_ref)
            for t in range(NX):
                layernorm(t)
            for c in w_copies():
                c.start()

        @pl.when(p + 1 < NP)
        def _():
            for c in b_copies(p + 1, 1 - slot):
                c.start()

        @pl.when(p == ffn_step)
        def _():
            route_and_ffn()

        for c in b_copies(p, slot):
            c.wait()

        step()

        @pl.when(p == NP - 1)
        def _():
            for t in range(NO):
                epilogue(t)
            for t in range(NO):
                o_copy(t).wait()

    @jax.jit
    def run(A_x, A_k_cache, A_v_cache, A_wq, A_wo, B_x, B_w_r, B_w_gate, B_w_up, B_w_down):
        x = A_x.reshape(S, D)
        kt = jnp.swapaxes(A_k_cache, 2, 3).reshape(H, DH, S)
        vt = jnp.swapaxes(A_v_cache, 2, 3).reshape(H, DH, S)
        wr = B_w_r if WR1D else B_w_r.reshape(1, D)
        anyspec = pl.BlockSpec(memory_space=pl.ANY)
        out = pl.pallas_call(
            kernel,
            grid=(NP,),
            in_specs=[anyspec, anyspec, anyspec, anyspec, anyspec,
                      pl.BlockSpec((D,), lambda p: (0,)) if WR1D else pl.BlockSpec((1, D), lambda p: (0, 0)),
                      anyspec, anyspec, anyspec],
            out_specs=anyspec,
            out_shape=jax.ShapeDtypeStruct((S, D), bf16),
            scratch_shapes=[
                pltpu.VMEM((S, D), bf16),
                pltpu.VMEM((S, D), bf16),
                pltpu.VMEM((S, D), bf16),
                pltpu.VMEM((D, S), f32),
                pltpu.VMEM((2, G, DH, W), bf16),
                pltpu.VMEM((2, G, DH, W), bf16),
                pltpu.VMEM((2, D, G * DH), bf16),
                pltpu.VMEM((2, G * DH, D), bf16),
                pltpu.VMEM((G, W, 256), bf16),
                pltpu.VMEM((D, G * DH), bf16),
                pltpu.VMEM((NX, 8, 128), f32),
                pltpu.VMEM((D, F), bf16),
                pltpu.VMEM((D, F), bf16),
                pltpu.VMEM((F, D), bf16),
                pltpu.VMEM((S, D), bf16),
                pltpu.SemaphoreType.DMA((NX,)),
                pltpu.SemaphoreType.DMA((2, 4)),
                pltpu.SemaphoreType.DMA((3,)),
                pltpu.SemaphoreType.DMA((NO,)),
            ],
            compiler_params=pltpu.CompilerParams(
                dimension_semantics=("arbitrary",),
                vmem_limit_bytes=vmem_mb * 1024 * 1024, flags=flags),
        )(x, kt, vt, A_wq, A_wo, wr, B_w_gate, B_w_up, B_w_down)
        return out.reshape(1, S, D)

    return run


pallas_recurrent_scan__sliding_block_cached__moe_arch_mod__prompt_kernel = make_kernel(
    flags={"XLA_TPU_FORCE_LP_LLO_SCHEDULER": True})
```

```python
import jax
import jax.numpy as jnp
from jax import lax
import jax.experimental.pallas as pl
import jax.experimental.pallas.tpu as pltpu

S = 2048
D = 640
H = 32
DH = 192
W = 512
F = 1536
G = 2
NP = H // G
LOG2E = 1.4426950408889634

bf16 = jnp.bfloat16
f32 = jnp.float32

NT = (((1,), (1,)), ((), ()))


def _sigmoid(x):
    e = jnp.exp(jnp.minimum(-x, 80.0))
    d = 1.0 + e
    r = pl.reciprocal(d, approx=True)
    return r * (2.0 - d * r)


def make_kernel(TQ=1024, vmem_mb=100, sched=None, TX=512, RC=512, TO=256, ffn_step=1, flags=None, LNU=1, WR1D=False, dmaord=1, wlate=False):
    NQ = S // TQ
    NX = S // TX
    NO = S // TO

    def kernel(x_hbm, kt_hbm, vt_hbm, wq_hbm, wo_hbm, wr_ref, wg_hbm, wu_hbm, wd_hbm,
               o_hbm, x_scr, xn_ref, g_scr, acc_ref, kt_buf, vt_buf, wq_buf, wo_buf, k_scr, wot_scr,
               r_scr, wg_scr, wu_scr, wd_scr, o_scr, xsem, bsem, wsem, osem):
        p = pl.program_id(0)
        slot = p % 2

        def x_copy(t):
            return pltpu.make_async_copy(x_hbm.at[pl.ds(t * TX, TX)], x_scr.at[pl.ds(t * TX, TX)], xsem.at[t])

        def o_copy(t):
            return pltpu.make_async_copy(o_scr.at[pl.ds(t * TO, TO)], o_hbm.at[pl.ds(t * TO, TO)], osem.at[t])

        def w_copies():
            return [pltpu.make_async_copy(a, b, wsem.at[i])
                    for i, (a, b) in enumerate(((wg_hbm, wg_scr), (wu_hbm, wu_scr), (wd_hbm, wd_scr)))]

        def b_copies(q, s):
            hs = pl.ds(q * G, G)
            cs = pl.ds(pl.multiple_of(q * (G * DH), G * DH), G * DH)
            ws = pl.ds(S - W, W)
            return [
                pltpu.make_async_copy(wq_hbm.at[:, cs], wq_buf.at[s], bsem.at[s, 0]),
                pltpu.make_async_copy(kt_hbm.at[hs, :, ws], kt_buf.at[s], bsem.at[s, 1]),
                pltpu.make_async_copy(vt_hbm.at[hs, :, ws], vt_buf.at[s], bsem.at[s, 2]),
                pltpu.make_async_copy(wo_hbm.at[cs, :], wo_buf.at[s], bsem.at[s, 3]),
            ]

        def layernorm(t):
            x_copy(t).wait()
            wr = wr_ref[...].astype(f32).reshape(1, D)
            lane = lax.broadcasted_iota(jnp.int32, (8, 128), 1)

            def body(c, rm):
                rows = pl.ds(pl.multiple_of(t * TX + c * RC, RC), RC)
                x = x_scr[rows, :].astype(f32)
                m = jnp.mean(x, axis=-1, keepdims=True)
                xc = x - m
                v = jnp.mean(xc * xc, axis=-1, keepdims=True)
                xn = xc * lax.rsqrt(v + 1e-5)
                xn_ref[rows, :] = xn.astype(bf16)
                h = 0.5 * xn
                g_scr[rows, :] = (h + h * jnp.tanh(h)).astype(bf16)
                r = jnp.sum(xn * wr, axis=-1, keepdims=True)
                for j in range(RC // 8):
                    rm = jnp.where(lane == c * (RC // 8) + j, r[8 * j:8 * j + 8, :], rm)
                return rm

            r_scr[t] = lax.fori_loop(0, TX // RC, body, jnp.full((8, 128), -jnp.inf, f32), unroll=LNU)

        def route():
            r = r_scr[...]
            shp = (NX, 8, 128)
            row = (lax.broadcasted_iota(jnp.int32, shp, 0) * TX
                   + lax.broadcasted_iota(jnp.int32, shp, 2) * 8
                   + lax.broadcasted_iota(jnp.int32, shp, 1))
            m1 = jnp.max(r)
            i1 = jnp.min(jnp.where(r == m1, row, S - 1))
            r2 = jnp.where(row == i1, -jnp.inf, r)
            m2 = jnp.max(r2)
            i2 = jnp.min(jnp.where(r2 == m2, row, S - 1))
            return i1, i2, m1, m2

        def ffn(i1, i2, m1, m2):
            for c in w_copies():
                c.wait()
            sub = lax.broadcasted_iota(jnp.int32, (16, 1), 0)
            a1 = pl.multiple_of((i1 // 16) * 16, 16)
            a2 = pl.multiple_of((i2 // 16) * 16, 16)
            c1 = xn_ref[pl.ds(a1, 16), :].astype(f32)
            c2 = xn_ref[pl.ds(a2, 16), :].astype(f32)
            x1 = jnp.sum(jnp.where(sub == i1 - a1, c1, 0.0), axis=0, keepdims=True)
            x2 = jnp.sum(jnp.where(sub == i2 - a2, c2, 0.0), axis=0, keepdims=True)
            xs = jnp.where(sub == 0, x1, jnp.where(sub == 1, x2, 0.0)).astype(bf16)
            gt = jnp.dot(xs, wg_scr[...], preferred_element_type=f32)
            up = jnp.dot(xs, wu_scr[...], preferred_element_type=f32)
            hmid = (gt * _sigmoid(gt) * up).astype(bf16)
            y = jnp.dot(hmid, wd_scr[...], preferred_element_type=f32)
            y = y * _sigmoid(jnp.where(sub == 0, m1, m2))
            y1 = y[0:1, :]
            y2 = y[1:2, :]
            for a, c in ((a1, c1), (a2, c2)):
                z = c + jnp.where(sub + a == i1, y1, jnp.where(sub + a == i2, y2, 0.0))
                g_scr[pl.ds(a, 16), :] = (z * _sigmoid(z)).astype(bf16)

        def epilogue(t):
            off = t * TO if isinstance(t, int) else pl.multiple_of(t * TO, TO)
            rows = pl.ds(off, TO)
            s = acc_ref[:, rows].astype(bf16).T.astype(f32)
            x = x_scr[rows, :].astype(f32)
            o_scr[rows, :] = (x + s * g_scr[rows, :].astype(f32)).astype(bf16)

        def o_start(t):
            off = pl.multiple_of(t * TO, TO)
            pltpu.make_async_copy(o_scr.at[pl.ds(off, TO)], o_hbm.at[pl.ds(off, TO)], osem.at[t]).start()

        qscale = (DH ** -0.5) * LOG2E

        def step():
            def sl(t):
                return pl.ds(t * TQ, TQ)

            def qproj(t):
                return (jnp.dot(xn_ref[sl(t), :], wq_buf[slot], preferred_element_type=f32) * qscale).astype(bf16)

            def qk(q, h):
                return lax.dot_general(k_scr[h], q[:, 128 * h:128 * h + 256], NT, preferred_element_type=f32)

            def sm(st):
                mx = jnp.max(st, axis=0, keepdims=True)
                pt = jnp.exp2(st - mx)
                l = jnp.sum(pt, axis=0, keepdims=True)
                return pt.astype(bf16), 1.0 / l

            def pv(pl_, h):
                pt, rl = pl_
                return (jnp.dot(vt_buf[slot, h], pt, preferred_element_type=f32) * rl).astype(bf16)

            def oproj(t, o0, o1):
                ot2 = jnp.concatenate([o0, o1], axis=0)
                acc_ref[:, sl(t)] += jnp.dot(wot_scr[...], ot2, preferred_element_type=f32)

            sc = sched
            if sc is None:
                sc = [("TK", 0), ("TK", 1), ("TW",)]
                for t in range(NQ):
                    sc += [("Q", t), ("K", t, 0), ("K", t, 1), ("S", t, 0), ("P", t, 0), ("S", t, 1), ("P", t, 1), ("O", t)]
            v = {}
            for tok in sc:
                k = tok[0]
                if k == "TK":
                    z = jnp.zeros((64, W), bf16)
                    h = tok[1]
                    k_scr[h] = (jnp.concatenate([kt_buf[slot, 0], z], axis=0) if h == 0
                                else jnp.concatenate([z, kt_buf[slot, 1]], axis=0)).T
                elif k == "TW":
                    wot_scr[...] = wo_buf[slot].T
                elif k == "Q":
                    v[tok] = qproj(tok[1])
                elif k == "K":
                    v[tok] = qk(v[("Q", tok[1])], tok[2])
                elif k == "S":
                    v[tok] = sm(v[("K",) + tok[1:]])
                elif k == "P":
                    v[tok] = pv(v[("S",) + tok[1:]], tok[2])
                elif k == "O":
                    oproj(tok[1], v[("P", tok[1], 0)], v[("P", tok[1], 1)])

        @pl.when(p == 0)
        def _():
            for t in range(NX):
                x_copy(t).start()
            if dmaord == 0:
                for c in b_copies(0, 0):
                    c.start()
            acc_ref[...] = jnp.zeros_like(acc_ref)
            for t in range(NX):
                layernorm(t)
                if dmaord == t + 1:
                    for c in b_copies(0, 0):
                        c.start()
            if not wlate:
                for c in w_copies():
                    c.start()

        if wlate:
            @pl.when(p == 1)
            def _():
                for c in w_copies():
                    c.start()

        @pl.when(p + 1 < NP)
        def _():
            for c in b_copies(p + 1, 1 - slot):
                c.start()

        for c in b_copies(p, slot):
            c.wait()

        step()

        @pl.when(p == NP - 1)
        def _():
            i1, i2, m1, m2 = route()
            c1 = i1 // TO
            c2 = i2 // TO
            for t in range(NO):
                epilogue(t)

                @pl.when(jnp.logical_and(c1 != t, c2 != t))
                def _():
                    o_copy(t).start()
            ffn(i1, i2, m1, m2)
            epilogue(c1)
            o_start(c1)

            @pl.when(c2 != c1)
            def _():
                epilogue(c2)
                o_start(c2)
            for t in range(NO):
                o_copy(t).wait()

    @jax.jit
    def run(A_x, A_k_cache, A_v_cache, A_wq, A_wo, B_x, B_w_r, B_w_gate, B_w_up, B_w_down):
        x = A_x.reshape(S, D)
        kt = jnp.swapaxes(A_k_cache, 2, 3).reshape(H, DH, S)
        vt = jnp.swapaxes(A_v_cache, 2, 3).reshape(H, DH, S)
        wr = B_w_r if WR1D else B_w_r.reshape(1, D)
        anyspec = pl.BlockSpec(memory_space=pl.ANY)
        out = pl.pallas_call(
            kernel,
            grid=(NP,),
            in_specs=[anyspec, anyspec, anyspec, anyspec, anyspec,
                      pl.BlockSpec((D,), lambda p: (0,)) if WR1D else pl.BlockSpec((1, D), lambda p: (0, 0)),
                      anyspec, anyspec, anyspec],
            out_specs=anyspec,
            out_shape=jax.ShapeDtypeStruct((S, D), bf16),
            scratch_shapes=[
                pltpu.VMEM((S, D), bf16),
                pltpu.VMEM((S, D), bf16),
                pltpu.VMEM((S, D), bf16),
                pltpu.VMEM((D, S), f32),
                pltpu.VMEM((2, G, DH, W), bf16),
                pltpu.VMEM((2, G, DH, W), bf16),
                pltpu.VMEM((2, D, G * DH), bf16),
                pltpu.VMEM((2, G * DH, D), bf16),
                pltpu.VMEM((G, W, 256), bf16),
                pltpu.VMEM((D, G * DH), bf16),
                pltpu.VMEM((NX, 8, 128), f32),
                pltpu.VMEM((D, F), bf16),
                pltpu.VMEM((D, F), bf16),
                pltpu.VMEM((F, D), bf16),
                pltpu.VMEM((S, D), bf16),
                pltpu.SemaphoreType.DMA((NX,)),
                pltpu.SemaphoreType.DMA((2, 4)),
                pltpu.SemaphoreType.DMA((3,)),
                pltpu.SemaphoreType.DMA((NO,)),
            ],
            compiler_params=pltpu.CompilerParams(
                dimension_semantics=("arbitrary",),
                vmem_limit_bytes=vmem_mb * 1024 * 1024, flags=flags),
        )(x, kt, vt, A_wq, A_wo, wr, B_w_gate, B_w_up, B_w_down)
        return out.reshape(1, S, D)

    return run


pallas_recurrent_scan__sliding_block_cached__moe_arch_mod__prompt_kernel = make_kernel(
    flags={"XLA_TPU_FORCE_LP_LLO_SCHEDULER": True})
```
